```python
import os as _os
_os.environ.setdefault('JAX_PLATFORMS', 'cpu')
import jax
import jax.numpy as jnp

def _softmax(x, axis=-1):
    return jax.nn.softmax(x, axis=axis)

def _gelu(x):
    return jax.nn.gelu(x, approximate=True)

def _silu(x):
    return jax.nn.silu(x)

def _sigmoid(x):
    return jax.nn.sigmoid(x)

def _layernorm(x, axis=-1, eps=1e-05):
    m = jnp.mean(x, axis=axis, keepdims=True)
    v = jnp.var(x, axis=axis, keepdims=True)
    return (x - m) / jnp.sqrt(v + eps)

def _scatter_add(tgt, idx, src, axis=0):
    return tgt.at[idx].add(src)

def _segment_sum(src, seg, n):
    return jax.ops.segment_sum(src, seg, n)

class _Rng:

    def __init__(self, key):
        self._k = key

    def _next(self):
        self._k, sub = jax.random.split(self._k)
        return sub

    def normal(self, shape):
        return jax.random.normal(self._next(), shape, dtype=jnp.bfloat16)

    def randint(self, lo, hi, shape):
        return jax.random.randint(self._next(), shape, lo, hi, dtype=jnp.int32)

    def uniform(self, shape, lo=0.0, hi=1.0):
        return jax.random.uniform(self._next(), shape, jnp.bfloat16, lo, hi)

    def permutation(self, n):
        return jax.random.permutation(self._next(), n)
kernel_name = 'parallel_sum__memory_aug_recurrent_mem_tr__dense_activation_silu__prompt'

def setup_inputs():
    _rng = _Rng(jax.random.key(int.from_bytes(__import__("os").urandom(4), "little")))
    _w = lambda a: (lambda t: t.astype(jnp.bfloat16) if jnp.issubdtype(t.dtype, jnp.floating) else t)(jnp.asarray(a))

    def _A_setup():
        B, S, Dm = (1, 2048, 448)
        H, Dh = (16, 256)
        M, seg = (8, 32)
        seg = min(seg, S)
        S = S // seg * seg
        return {'x': _w((lambda *s: _rng.normal(s) * 0.05)(B, S, Dm)), 'mem0': _w((lambda *s: _rng.normal(s) * 0.2)(B, M, Dm)), 'Wq': _w((lambda *s: _rng.normal(s) * 0.8)(Dm, H, Dh) * Dm ** (-0.5)), 'Wk': _w((lambda *s: _rng.normal(s) * 0.8)(Dm, H, Dh) * Dm ** (-0.5)), 'Wv': _w((lambda *s: _rng.normal(s) * 0.2)(Dm, H, Dh) * Dm ** (-0.5)), 'Wo': _w((lambda *s: _rng.normal(s) * 0.2)(H, Dh, Dm) * (H * Dh) ** (-0.5)), 'seg_len': seg}
    _A_in = _A_setup()

    def _B_setup():
        B, S, D, F = (1, 2048, 448, 1792)
        return {'x': _w((lambda *s: _rng.normal(s) * 0.05)(B, S, D)), 'w1': _w((lambda *s: _rng.normal(s) * 0.05)(D, F) * D ** (-0.5)), 'w2': _w((lambda *s: _rng.normal(s) * 0.05)(F, D) * F ** (-0.5))}
    _B_in = _B_setup()
    return {'A_x': _A_in['x'], 'A_mem0': _A_in['mem0'], 'A_Wq': _A_in['Wq'], 'A_Wk': _A_in['Wk'], 'A_Wv': _A_in['Wv'], 'A_Wo': _A_in['Wo'], 'A_seg_len': _A_in['seg_len'], 'B_x': _B_in['x'], 'B_w1': _B_in['w1'], 'B_w2': _B_in['w2']}

def reference(A_x, A_mem0, A_Wq, A_Wk, A_Wv, A_Wo, A_seg_len, B_x, B_w1, B_w2):

    def _A_ref(x, mem0, Wq, Wk, Wv, Wo, seg_len):
        B, S, Dm = x.shape
        H, Dh = (Wq.shape[1], Wq.shape[2])
        M = mem0.shape[1]
        scale = Dh ** (-0.5)
        n_seg = S // seg_len
        L = M + seg_len
        idx = jnp.arange(L)
        mask = (idx[:, None] < M) | (idx[:, None] >= idx[None, :])
        mem = mem0
        outs = []
        for s in range(n_seg):
            xs = x[:, s * seg_len:(s + 1) * seg_len, :].copy()
            h = jnp.concatenate([mem, xs], axis=1)
            q = jnp.einsum('btd,dhe->bhte', h, Wq)
            k = jnp.einsum('btd,dhe->bhte', h, Wk)
            v = jnp.einsum('btd,dhe->bhte', h, Wv)
            scores = jnp.einsum('bhqe,bhke->bhqk', q, k) * scale
            scores = jnp.where(mask[None, None], scores, -1000000000.0)
            p = _softmax(scores, axis=-1)
            o = jnp.einsum('bhqk,bhke->bhqe', p, v)
            o = jnp.einsum('bhte,hed->btd', o, Wo)
            mem = o[:, :M, :].copy()
            outs.append(o[:, M:, :])
        return jnp.concatenate(outs, axis=1)

    def _B_ref(x, w1, w2):
        h = jnp.einsum('bsd,df->bsf', x, w1)
        h = _silu(h)
        out = jnp.einsum('bsf,fd->bsd', h, w2)
        return out
    x = A_x
    xn = _layernorm(x, axis=-1)
    return x + _A_ref(xn, A_mem0, A_Wq, A_Wk, A_Wv, A_Wo, A_seg_len) + _B_ref(xn, B_w1, B_w2)
```

```python
import functools
import jax
import jax.numpy as jnp
from jax import lax
import jax.experimental.pallas as pl
import jax.experimental.pallas.tpu as pltpu

_F32 = jnp.float32
_BF16 = jnp.bfloat16


def _kernel(x_ref, mem0_ref, wq_ref, wk_ref, wv_ref, wo_ref, w1_ref, w2_ref,
            o_ref, mem_sc, wq_s, wk_s, wv_s, wo_s, w1_s, w2_s, *, n_heads, head_dim, n_mem, seg_len, eps):
    step = pl.program_id(0)

    @pl.when(step == 0)
    def _():
        mem_sc[...] = mem0_ref[...].astype(_F32)
        wq_s[...] = pltpu.bitcast(wq_ref[...], jnp.int32)
        wk_s[...] = pltpu.bitcast(wk_ref[...], jnp.int32)
        wv_s[...] = pltpu.bitcast(wv_ref[...], jnp.int32)
        wo_s[...] = pltpu.bitcast(wo_ref[...], jnp.int32)
        w1_s[...] = pltpu.bitcast(w1_ref[...], jnp.int32)
        w2_s[...] = pltpu.bitcast(w2_ref[...], jnp.int32)

    M, T = n_mem, seg_len
    L = M + T
    SP = 8
    LP = L + SP
    LS = L - SP
    T0 = T - SP
    scale = float(head_dim) ** (-0.5)
    n_pairs = n_heads // 2

    xf = x_ref[...].astype(_F32)
    mu = jnp.mean(xf, axis=-1, keepdims=True)
    xc = xf - mu
    var = jnp.mean(xc * xc, axis=-1, keepdims=True)
    xn = xc * lax.rsqrt(var + eps)
    xn_b = xn.astype(_BF16)
    xa, xb = xn[:T], xn[T:]

    r = lax.broadcasted_iota(jnp.int32, (LP, LP), 0)
    c = lax.broadcasted_iota(jnp.int32, (LP, LP), 1)
    pos_r = jnp.where(r >= L, r - SP, r)
    pos_c = jnp.where(c >= L, c - SP, c)
    mask_a = ((c < LS) | (c >= L)) & ((r < M) | (pos_r >= pos_c))
    mask_b = (c < L) & ((r < M) | (r >= c))

    def scores(qf, kf, hd):
        sl = slice(hd * head_dim, (hd + 1) * head_dim)
        return lax.dot_general(qf[:, sl], kf[:, sl], (((1,), (1,)), ((), ())),
                               preferred_element_type=_F32)

    def softmax(s, mask):
        s = jnp.where(mask, s, -1000000000.0)
        m = jnp.max(s, axis=-1, keepdims=True)
        p = jnp.exp(s - m)
        l = jnp.sum(p, axis=-1, keepdims=True)
        return (p / l).astype(_BF16)

    def attention(qf, kf, v_lhs, v_extra, mask):
        outs, v_tails, pend = [], [], None
        for hp in range(n_pairs + 1):
            if hp < n_pairs:
                s_a = scores(qf, kf, 2 * hp)
                s_b = scores(qf, kf, 2 * hp + 1)
                sl2 = slice(2 * hp * head_dim, (2 * hp + 2) * head_dim)
                v_pair = jnp.dot(v_lhs, pltpu.bitcast(wv_s[:, sl2], _BF16), preferred_element_type=_F32).astype(_BF16)
                if v_extra is None:
                    v_tails.append(v_pair[LS:LP])
                else:
                    v_pair = jnp.concatenate([v_pair, v_extra[hp]], axis=0)
                p_a = softmax(s_a, mask)
                p_b = softmax(s_b, mask)
            if pend is not None:
                pa, pb, vp = pend
                outs.append(jnp.dot(pa, vp[:, :head_dim], preferred_element_type=_F32))
                outs.append(jnp.dot(pb, vp[:, head_dim:], preferred_element_type=_F32))
            pend = (p_a, p_b, v_pair) if hp < n_pairs else None
        return outs, v_tails

    hA = jnp.concatenate([mem_sc[...], xa[:T0], xb[T0:], xa[T0:]], axis=0).astype(_BF16)
    qA = (jnp.dot(hA, pltpu.bitcast(wq_s[...], _BF16), preferred_element_type=_F32) * scale).astype(_BF16)
    kA = jnp.dot(hA, pltpu.bitcast(wk_s[...], _BF16), preferred_element_type=_F32).astype(_BF16)
    oA, vA_tails = attention(qA, kA, hA, None, mask_a)

    oA_lhs = jnp.concatenate([o[:LS].astype(_BF16) for o in oA], axis=1)
    yA = jnp.dot(oA_lhs, pltpu.bitcast(wo_s[...], _BF16), preferred_element_type=_F32)
    mem_b = yA[:M].astype(_BF16).astype(_F32)
    mem_sc[...] = mem_b

    f = jnp.dot(xn_b, pltpu.bitcast(w1_s[...], _BF16), preferred_element_type=_F32)
    f = (f * jax.nn.sigmoid(f)).astype(_BF16)

    hB = jnp.concatenate([mem_b, xb[:T0]], axis=0).astype(_BF16)
    qB = (jnp.dot(hB, pltpu.bitcast(wq_s[...], _BF16), preferred_element_type=_F32) * scale).astype(_BF16)
    kB = jnp.dot(hB, pltpu.bitcast(wk_s[...], _BF16), preferred_element_type=_F32).astype(_BF16)
    q_b = jnp.concatenate([qB, qA[LS:LP]], axis=0)
    k_b = jnp.concatenate([kB, kA[LS:LP]], axis=0)
    oB, _ = attention(q_b, k_b, hB, vA_tails, mask_b)

    oB_lhs = jnp.concatenate(
        [jnp.concatenate([ob[:L], oa[L:LP]], axis=0).astype(_BF16) for oa, ob in zip(oA, oB)],
        axis=1)
    yB = jnp.dot(oB_lhs, pltpu.bitcast(wo_s[...], _BF16), preferred_element_type=_F32)

    g = jnp.dot(f, pltpu.bitcast(w2_s[...], _BF16), preferred_element_type=_F32)

    mem_sc[...] = yB[:M].astype(_BF16).astype(_F32)
    attn = jnp.concatenate([yA[M:LS], yB[L:LP], yB[M:L]], axis=0)
    o_ref[...] = (xf + attn + g).astype(o_ref.dtype)


@functools.partial(jax.jit, static_argnames=("A_seg_len",))
def pallas_parallel_sum__memory_aug_recurrent_mem_tr__dense_activation_silu__prompt_kernel(
    A_x, A_mem0, A_Wq, A_Wk, A_Wv, A_Wo, A_seg_len, B_x, B_w1, B_w2):
    del B_x
    B, S, D = A_x.shape
    _, H, Dh = A_Wq.shape
    M = A_mem0.shape[1]
    seg = int(A_seg_len)
    n_seg = S // seg
    F = B_w1.shape[1]
    assert B == 1 and S % seg == 0 and n_seg % 2 == 0 and H % 2 == 0
    assert M % 8 == 0 and seg % 8 == 0 and seg >= 8 and (M + seg) % 16 == 8
    x2 = A_x.reshape(S, D)
    mem0 = A_mem0.reshape(M, D)
    wq = A_Wq.reshape(D, H * Dh)
    wk = A_Wk.reshape(D, H * Dh)
    wv = A_Wv.reshape(D, H * Dh)
    wo = A_Wo.reshape(H * Dh, D)
    const = lambda shape: pl.BlockSpec(shape, lambda s: (0, 0))
    kernel = functools.partial(_kernel, n_heads=H, head_dim=Dh, n_mem=M, seg_len=seg, eps=1e-05)
    out = pl.pallas_call(
        kernel, grid=(n_seg // 2,),
        in_specs=[pl.BlockSpec((2 * seg, D), lambda s: (s, 0)), const((M, D)),
                  const((D, H * Dh)), const((D, H * Dh)), const((D, H * Dh)), const((H * Dh, D)),
                  const((D, F)), const((F, D))],
        out_specs=pl.BlockSpec((2 * seg, D), lambda s: (s, 0)),
        out_shape=jax.ShapeDtypeStruct((S, D), A_x.dtype),
        scratch_shapes=[pltpu.VMEM((M, D), _F32),
                        pltpu.VMEM((D // 2, H * Dh), jnp.int32), pltpu.VMEM((D // 2, H * Dh), jnp.int32),
                        pltpu.VMEM((D // 2, H * Dh), jnp.int32), pltpu.VMEM((H * Dh // 2, D), jnp.int32),
                        pltpu.VMEM((D // 2, F), jnp.int32), pltpu.VMEM((F // 2, D), jnp.int32)],
        compiler_params=pltpu.CompilerParams(dimension_semantics=("arbitrary",), vmem_limit_bytes=100 * 1024 * 1024),
    )(x2, mem0, wq, wk, wv, wo, B_w1, B_w2)
    return out.reshape(B, S, D)
```

```python
import functools
import jax
import jax.numpy as jnp
from jax import lax
import jax.experimental.pallas as pl
import jax.experimental.pallas.tpu as pltpu

_F32 = jnp.float32
_BF16 = jnp.bfloat16


def _kernel(x_ref, xnext_ref, mem0_ref, wq_ref, wk_ref, wv_ref, wo_ref, w1_ref, w2T_ref,
            o_ref, mem_sc, xn_sc, g_sc, wq_s, wk_s, wv_s, wo_s, w1_s, w2T_s, *, n_heads, head_dim, n_mem, seg_len, eps):
    step = pl.program_id(0)

    def layernorm(ref):
        v = ref[...].astype(_F32)
        mu = jnp.mean(v, axis=-1, keepdims=True)
        vc = v - mu
        var = jnp.mean(vc * vc, axis=-1, keepdims=True)
        return vc * lax.rsqrt(var + eps)

    def ffn1(xn_val):
        f = jnp.dot(xn_val.astype(_BF16), pltpu.bitcast(w1_s[...], _BF16), preferred_element_type=_F32)
        return (f * jax.nn.sigmoid(f)).astype(_BF16)

    def ffn2(f):
        return lax.dot_general(f, pltpu.bitcast(w2T_s[...], _BF16), (((1,), (1,)), ((), ())),
                               preferred_element_type=_F32)

    FC = 256
    n_fc = w1_s.shape[1] // FC

    def ffn1_chunk(xn_bf, i):
        f = jnp.dot(xn_bf, pltpu.bitcast(w1_s[:, i * FC:(i + 1) * FC], _BF16), preferred_element_type=_F32)
        return (f * jax.nn.sigmoid(f)).astype(_BF16)

    def ffn2_chunk(f_chunk, i):
        return lax.dot_general(f_chunk, pltpu.bitcast(w2T_s[:, i * FC:(i + 1) * FC], _BF16),
                               (((1,), (1,)), ((), ())), preferred_element_type=_F32)

    @pl.when(step == 0)
    def _():
        mem_sc[...] = mem0_ref[...].astype(_F32)
        wq_s[...] = pltpu.bitcast(wq_ref[...], jnp.int32)
        wk_s[...] = pltpu.bitcast(wk_ref[...], jnp.int32)
        wv_s[...] = pltpu.bitcast(wv_ref[...], jnp.int32)
        wo_s[...] = pltpu.bitcast(wo_ref[...], jnp.int32)
        w1_s[...] = pltpu.bitcast(w1_ref[...], jnp.int32)
        w2T_s[...] = pltpu.bitcast(w2T_ref[...], jnp.int32)
        xn0 = layernorm(x_ref)
        xn_sc[...] = xn0
        g_sc[...] = ffn2(ffn1(xn0))

    M, T = n_mem, seg_len
    L = M + T
    SP = 8
    LP = L + SP
    LS = L - SP
    T0 = T - SP
    scale = float(head_dim) ** (-0.5)
    n_pairs = n_heads // 2

    xf = x_ref[...].astype(_F32)
    xn = xn_sc[...]
    g_cur = g_sc[...]
    xa, xb = xn[:T], xn[T:]

    r = lax.broadcasted_iota(jnp.int32, (LP, LP), 0)
    c = lax.broadcasted_iota(jnp.int32, (LP, LP), 1)
    pos_r = jnp.where(r >= L, r - SP, r)
    pos_c = jnp.where(c >= L, c - SP, c)
    mask_a = ((c < LS) | (c >= L)) & ((r < M) | (pos_r >= pos_c))
    mask_b = (c < L) & ((r < M) | (r >= c))

    def scores(qf, kf, hd):
        sl = slice(hd * head_dim, (hd + 1) * head_dim)
        return lax.dot_general(qf[:, sl], kf[:, sl], (((1,), (1,)), ((), ())),
                               preferred_element_type=_F32)

    def softmax(s, mask):
        s = jnp.where(mask, s, -1000000000.0)
        m = jnp.max(s, axis=-1, keepdims=True)
        p = jnp.exp(s - m)
        l = jnp.sum(p, axis=-1, keepdims=True)
        return (p / l).astype(_BF16)

    def attention(qf, kf, v_lhs, v_extra, mask, fillers=None):
        SKEW = 2
        outs, v_tails, pend = [], [], []
        for hp in range(n_pairs + SKEW):
            if hp < n_pairs:
                s_a = scores(qf, kf, 2 * hp)
                s_b = scores(qf, kf, 2 * hp + 1)
                sl2 = slice(2 * hp * head_dim, (2 * hp + 2) * head_dim)
                v_pair = jnp.dot(v_lhs, pltpu.bitcast(wv_s[:, sl2], _BF16), preferred_element_type=_F32).astype(_BF16)
                if v_extra is None:
                    v_tails.append(v_pair[LS:LP])
                else:
                    v_pair = jnp.concatenate([v_pair, v_extra[hp]], axis=0)
                p_a = softmax(s_a, mask)
                p_b = softmax(s_b, mask)
                pend.append((p_a, p_b, v_pair))
            if fillers is not None and hp in fillers:
                fillers[hp]()
            if hp >= SKEW:
                pa, pb, vp = pend[hp - SKEW]
                outs.append(jnp.dot(pa, vp[:, :head_dim], preferred_element_type=_F32))
                outs.append(jnp.dot(pb, vp[:, head_dim:], preferred_element_type=_F32))
        return outs, v_tails

    f_chunks = [None] * n_fc
    g_acc = [None]

    def do_ffn1(idx):
        for i in idx:
            f_chunks[i] = ffn1_chunk(xn_next_bf, i)

    def do_ffn2(idx):
        for i in idx:
            t = ffn2_chunk(f_chunks[i], i)
            g_acc[0] = t if g_acc[0] is None else g_acc[0] + t

    hA = jnp.concatenate([mem_sc[...], xa[:T0], xb[T0:], xa[T0:]], axis=0).astype(_BF16)
    qA = (jnp.dot(hA, pltpu.bitcast(wq_s[...], _BF16), preferred_element_type=_F32) * scale).astype(_BF16)
    xn_next = layernorm(xnext_ref)
    xn_sc[...] = xn_next
    xn_next_bf = xn_next.astype(_BF16)
    do_ffn1([0])
    kA = jnp.dot(hA, pltpu.bitcast(wk_s[...], _BF16), preferred_element_type=_F32).astype(_BF16)
    oA, vA_tails = attention(qA, kA, hA, None, mask_a,
                             fillers={n_pairs: lambda: do_ffn1([1]), n_pairs + 1: lambda: do_ffn1([2])})

    oA_lhs = jnp.concatenate([o[:LS].astype(_BF16) for o in oA], axis=1)
    yA = jnp.dot(oA_lhs, pltpu.bitcast(wo_s[...], _BF16), preferred_element_type=_F32)
    mem_b = yA[:M].astype(_BF16).astype(_F32)
    mem_sc[...] = mem_b
    do_ffn1([3, 4])

    hB = jnp.concatenate([mem_b, xb[:T0]], axis=0).astype(_BF16)
    qB = (jnp.dot(hB, pltpu.bitcast(wq_s[...], _BF16), preferred_element_type=_F32) * scale).astype(_BF16)
    do_ffn1([5, 6])
    kB = jnp.dot(hB, pltpu.bitcast(wk_s[...], _BF16), preferred_element_type=_F32).astype(_BF16)
    q_b = jnp.concatenate([qB, qA[LS:LP]], axis=0)
    k_b = jnp.concatenate([kB, kA[LS:LP]], axis=0)
    oB, _ = attention(q_b, k_b, hB, vA_tails, mask_b,
                      fillers={n_pairs: lambda: do_ffn2([0]), n_pairs + 1: lambda: do_ffn2([1, 2])})

    oB_lhs = jnp.concatenate(
        [jnp.concatenate([ob[:L], oa[L:LP]], axis=0).astype(_BF16) for oa, ob in zip(oA, oB)],
        axis=1)
    yB = jnp.dot(oB_lhs, pltpu.bitcast(wo_s[...], _BF16), preferred_element_type=_F32)

    do_ffn2(range(3, n_fc))
    g_next = g_acc[0]

    mem_sc[...] = yB[:M].astype(_BF16).astype(_F32)
    attn = jnp.concatenate([yA[M:LS], yB[L:LP], yB[M:L]], axis=0)
    o_ref[...] = (xf + attn + g_cur).astype(o_ref.dtype)
    g_sc[...] = g_next


@functools.partial(jax.jit, static_argnames=("A_seg_len",))
def pallas_parallel_sum__memory_aug_recurrent_mem_tr__dense_activation_silu__prompt_kernel(
    A_x, A_mem0, A_Wq, A_Wk, A_Wv, A_Wo, A_seg_len, B_x, B_w1, B_w2):
    del B_x
    B, S, D = A_x.shape
    _, H, Dh = A_Wq.shape
    M = A_mem0.shape[1]
    seg = int(A_seg_len)
    n_seg = S // seg
    F = B_w1.shape[1]
    assert B == 1 and S % seg == 0 and n_seg % 2 == 0 and H % 2 == 0
    assert M % 8 == 0 and seg % 8 == 0 and seg >= 8 and (M + seg) % 16 == 8
    x2 = A_x.reshape(S, D)
    mem0 = A_mem0.reshape(M, D)
    wq = A_Wq.reshape(D, H * Dh)
    wk = A_Wk.reshape(D, H * Dh)
    wv = A_Wv.reshape(D, H * Dh)
    wo = A_Wo.reshape(H * Dh, D)
    w2T = B_w2.T
    n_steps = n_seg // 2
    const = lambda shape: pl.BlockSpec(shape, lambda s: (0, 0))
    kernel = functools.partial(_kernel, n_heads=H, head_dim=Dh, n_mem=M, seg_len=seg, eps=1e-05)
    out = pl.pallas_call(
        kernel, grid=(n_steps,),
        in_specs=[pl.BlockSpec((2 * seg, D), lambda s: (s, 0)),
                  pl.BlockSpec((2 * seg, D), lambda s: (jnp.minimum(s + 1, n_steps - 1), 0)),
                  const((M, D)),
                  const((D, H * Dh)), const((D, H * Dh)), const((D, H * Dh)), const((H * Dh, D)),
                  const((D, F)), const((D, F))],
        out_specs=pl.BlockSpec((2 * seg, D), lambda s: (s, 0)),
        out_shape=jax.ShapeDtypeStruct((S, D), A_x.dtype),
        scratch_shapes=[pltpu.VMEM((M, D), _F32), pltpu.VMEM((2 * seg, D), _F32), pltpu.VMEM((2 * seg, D), _F32),
                        pltpu.VMEM((D // 2, H * Dh), jnp.int32), pltpu.VMEM((D // 2, H * Dh), jnp.int32),
                        pltpu.VMEM((D // 2, H * Dh), jnp.int32), pltpu.VMEM((H * Dh // 2, D), jnp.int32),
                        pltpu.VMEM((D // 2, F), jnp.int32), pltpu.VMEM((D // 2, F), jnp.int32)],
        compiler_params=pltpu.CompilerParams(dimension_semantics=("arbitrary",), vmem_limit_bytes=100 * 1024 * 1024),
    )(x2, x2, mem0, wq, wk, wv, wo, B_w1, w2T)
    return out.reshape(B, S, D)
```

```python
import functools
import jax
import jax.numpy as jnp
from jax import lax
import jax.experimental.pallas as pl
import jax.experimental.pallas.tpu as pltpu

_F32 = jnp.float32
_BF16 = jnp.bfloat16


def _kernel(x_ref, xnext_ref, mem0_ref, wq_ref, wk_ref, wv_ref, wo_ref, w1_ref, w2T_ref,
            o_ref, mem_sc, xn_sc, f0_sc, wq_s, wk_s, wv_s, wo_s, *, n_heads, head_dim, n_mem, seg_len, eps):
    step = pl.program_id(0)

    def layernorm(ref):
        v = ref[...].astype(_F32)
        mu = jnp.mean(v, axis=-1, keepdims=True)
        vc = v - mu
        var = jnp.mean(vc * vc, axis=-1, keepdims=True)
        return vc * lax.rsqrt(var + eps)

    FC = 256
    n_fc = w1_ref.shape[1] // FC

    def ffn1_chunk(xn_bf, i):
        f = jnp.dot(xn_bf, w1_ref[:, i * FC:(i + 1) * FC], preferred_element_type=_F32)
        return (f * jax.nn.sigmoid(f)).astype(_BF16)

    def ffn2_chunk(f_chunk, i):
        return lax.dot_general(f_chunk, w2T_ref[:, i * FC:(i + 1) * FC],
                               (((1,), (1,)), ((), ())), preferred_element_type=_F32)

    @pl.when(step == 0)
    def _():
        mem_sc[...] = mem0_ref[...].astype(_F32)
        wq_s[...] = pltpu.bitcast(wq_ref[...], jnp.int32)
        wk_s[...] = pltpu.bitcast(wk_ref[...], jnp.int32)
        wv_s[...] = pltpu.bitcast(wv_ref[...], jnp.int32)
        wo_s[...] = pltpu.bitcast(wo_ref[...], jnp.int32)
        xn0 = layernorm(x_ref)
        xn_sc[...] = xn0
        f0_sc[...] = ffn1_chunk(xn0.astype(_BF16), 0)

    M, T = n_mem, seg_len
    L = M + T
    SP = 8
    LP = L + SP
    LS = L - SP
    T0 = T - SP
    scale = float(head_dim) ** (-0.5)
    n_pairs = n_heads // 2

    xf = x_ref[...].astype(_F32)
    xn = xn_sc[...]
    xn_bf = xn.astype(_BF16)
    xa, xb = xn[:T], xn[T:]

    r = lax.broadcasted_iota(jnp.int32, (LP, LP), 0)
    c = lax.broadcasted_iota(jnp.int32, (LP, LP), 1)
    pos_r = jnp.where(r >= L, r - SP, r)
    pos_c = jnp.where(c >= L, c - SP, c)
    mask_a = ((c < LS) | (c >= L)) & ((r < M) | (pos_r >= pos_c))
    mask_b = (c < L) & ((r < M) | (r >= c))

    def scores(qf, kf, hd):
        sl = slice(hd * head_dim, (hd + 1) * head_dim)
        return lax.dot_general(qf[:, sl], kf[:, sl], (((1,), (1,)), ((), ())),
                               preferred_element_type=_F32)

    def softmax(s, mask):
        s = jnp.where(mask, s, -1000000000.0)
        m = jnp.max(s, axis=-1, keepdims=True)
        p = jnp.exp(s - m)
        l = jnp.sum(p, axis=-1, keepdims=True)
        return (p / l).astype(_BF16)

    def attention(qf, kf, v_lhs, v_extra, mask, fillers=None):
        SKEW = 2
        outs, v_tails, pend = [], [], []
        for hp in range(n_pairs + SKEW):
            if hp < n_pairs:
                s_a = scores(qf, kf, 2 * hp)
                s_b = scores(qf, kf, 2 * hp + 1)
                sl2 = slice(2 * hp * head_dim, (2 * hp + 2) * head_dim)
                v_pair = jnp.dot(v_lhs, pltpu.bitcast(wv_s[:, sl2], _BF16), preferred_element_type=_F32).astype(_BF16)
                if v_extra is None:
                    v_tails.append(v_pair[LS:LP])
                else:
                    v_pair = jnp.concatenate([v_pair, v_extra[hp]], axis=0)
                p_a = softmax(s_a, mask)
                p_b = softmax(s_b, mask)
                pend.append((p_a, p_b, v_pair))
            if fillers is not None and hp in fillers:
                fillers[hp]()
            if hp >= SKEW:
                pa, pb, vp = pend[hp - SKEW]
                outs.append(jnp.dot(pa, vp[:, :head_dim], preferred_element_type=_F32))
                outs.append(jnp.dot(pb, vp[:, head_dim:], preferred_element_type=_F32))
        return outs, v_tails

    f_chunks = [None] * n_fc
    g_acc = [None]

    def do_ffn1(idx):
        for i in idx:
            f_chunks[i] = ffn1_chunk(xn_bf, i)

    def do_ffn2(idx):
        for i in idx:
            t = ffn2_chunk(f_chunks[i], i)
            g_acc[0] = t if g_acc[0] is None else g_acc[0] + t

    hA = jnp.concatenate([mem_sc[...], xa[:T0], xb[T0:], xa[T0:]], axis=0).astype(_BF16)
    qA = (jnp.dot(hA, pltpu.bitcast(wq_s[...], _BF16), preferred_element_type=_F32) * scale).astype(_BF16)
    f_chunks[0] = f0_sc[...]
    xn_next = layernorm(xnext_ref)
    xn_sc[...] = xn_next
    f0_sc[...] = ffn1_chunk(xn_next.astype(_BF16), 0)
    kA = jnp.dot(hA, pltpu.bitcast(wk_s[...], _BF16), preferred_element_type=_F32).astype(_BF16)
    oA, vA_tails = attention(qA, kA, hA, None, mask_a,
                             fillers={n_pairs: lambda: do_ffn1([1]), n_pairs + 1: lambda: do_ffn1([2])})

    oA_lhs = jnp.concatenate([o[:LS].astype(_BF16) for o in oA], axis=1)
    yA = jnp.dot(oA_lhs, pltpu.bitcast(wo_s[...], _BF16), preferred_element_type=_F32)
    mem_b = yA[:M].astype(_BF16).astype(_F32)
    mem_sc[...] = mem_b
    do_ffn1([3, 4])

    hB = jnp.concatenate([mem_b, xb[:T0]], axis=0).astype(_BF16)
    qB = (jnp.dot(hB, pltpu.bitcast(wq_s[...], _BF16), preferred_element_type=_F32) * scale).astype(_BF16)
    do_ffn1([5, 6])
    kB = jnp.dot(hB, pltpu.bitcast(wk_s[...], _BF16), preferred_element_type=_F32).astype(_BF16)
    q_b = jnp.concatenate([qB, qA[LS:LP]], axis=0)
    k_b = jnp.concatenate([kB, kA[LS:LP]], axis=0)
    oB, _ = attention(q_b, k_b, hB, vA_tails, mask_b,
                      fillers={n_pairs: lambda: do_ffn2([0]), n_pairs + 1: lambda: do_ffn2([1, 2])})

    oB_lhs = jnp.concatenate(
        [jnp.concatenate([ob[:L], oa[L:LP]], axis=0).astype(_BF16) for oa, ob in zip(oA, oB)],
        axis=1)
    yB = jnp.dot(oB_lhs, pltpu.bitcast(wo_s[...], _BF16), preferred_element_type=_F32)

    do_ffn2(range(3, n_fc))
    g = g_acc[0]

    mem_sc[...] = yB[:M].astype(_BF16).astype(_F32)
    attn = jnp.concatenate([yA[M:LS], yB[L:LP], yB[M:L]], axis=0)
    o_ref[...] = (xf + attn + g).astype(o_ref.dtype)


@functools.partial(jax.jit, static_argnames=("A_seg_len",))
def pallas_parallel_sum__memory_aug_recurrent_mem_tr__dense_activation_silu__prompt_kernel(
    A_x, A_mem0, A_Wq, A_Wk, A_Wv, A_Wo, A_seg_len, B_x, B_w1, B_w2):
    del B_x
    B, S, D = A_x.shape
    _, H, Dh = A_Wq.shape
    M = A_mem0.shape[1]
    seg = int(A_seg_len)
    n_seg = S // seg
    F = B_w1.shape[1]
    assert B == 1 and S % seg == 0 and n_seg % 2 == 0 and H % 2 == 0
    assert M % 8 == 0 and seg % 8 == 0 and seg >= 8 and (M + seg) % 16 == 8
    assert F == 7 * 256 and D % 16 == 0 and Dh % 128 == 0
    x2 = A_x.reshape(S, D)
    mem0 = A_mem0.reshape(M, D)
    wq = A_Wq.reshape(D, H * Dh)
    wk = A_Wk.reshape(D, H * Dh)
    wv = A_Wv.reshape(D, H * Dh)
    wo = A_Wo.reshape(H * Dh, D)
    w2T = B_w2.T
    n_steps = n_seg // 2
    const = lambda shape: pl.BlockSpec(shape, lambda s: (0, 0))
    kernel = functools.partial(_kernel, n_heads=H, head_dim=Dh, n_mem=M, seg_len=seg, eps=1e-05)
    out = pl.pallas_call(
        kernel, grid=(n_steps,),
        in_specs=[pl.BlockSpec((2 * seg, D), lambda s: (s, 0)),
                  pl.BlockSpec((2 * seg, D), lambda s: (jnp.minimum(s + 1, n_steps - 1), 0)),
                  const((M, D)),
                  const((D, H * Dh)), const((D, H * Dh)), const((D, H * Dh)), const((H * Dh, D)),
                  const((D, F)), const((D, F))],
        out_specs=pl.BlockSpec((2 * seg, D), lambda s: (s, 0)),
        out_shape=jax.ShapeDtypeStruct((S, D), A_x.dtype),
        scratch_shapes=[pltpu.VMEM((M, D), _F32), pltpu.VMEM((2 * seg, D), _F32), pltpu.VMEM((2 * seg, 256), _BF16),
                        pltpu.VMEM((D // 2, H * Dh), jnp.int32), pltpu.VMEM((D // 2, H * Dh), jnp.int32),
                        pltpu.VMEM((D // 2, H * Dh), jnp.int32), pltpu.VMEM((H * Dh // 2, D), jnp.int32)],
        compiler_params=pltpu.CompilerParams(dimension_semantics=("arbitrary",), vmem_limit_bytes=100 * 1024 * 1024),
    )(x2, x2, mem0, wq, wk, wv, wo, B_w1, w2T)
    return out.reshape(B, S, D)
```
